```python
import os as _os
_os.environ.setdefault("JAX_PLATFORMS", "cpu")
import jax
import jax.numpy as jnp

def _softmax(x, axis=-1):
    return jax.nn.softmax(x, axis=axis)
def _gelu(x):
    return jax.nn.gelu(x, approximate=True)
def _silu(x):
    return jax.nn.silu(x)
def _sigmoid(x):
    return jax.nn.sigmoid(x)
def _layernorm(x, axis=-1, eps=1e-5):
    m = jnp.mean(x, axis=axis, keepdims=True)
    v = jnp.var(x, axis=axis, keepdims=True)
    return (x - m) / jnp.sqrt(v + eps)
def _scatter_add(tgt, idx, src, axis=0):
    return tgt.at[idx].add(src)
def _segment_sum(src, seg, n):
    return jax.ops.segment_sum(src, seg, n)
class _Rng:
    def __init__(self, key):
        self._k = key
    def _next(self):
        self._k, sub = jax.random.split(self._k)
        return sub
    def normal(self, shape):
        return jax.random.normal(self._next(), shape, dtype=jnp.bfloat16)
    def randint(self, lo, hi, shape):
        return jax.random.randint(self._next(), shape, lo, hi, dtype=jnp.int32)
    def uniform(self, shape, lo=0.0, hi=1.0):
        return jax.random.uniform(self._next(), shape, jnp.bfloat16, lo, hi)
    def permutation(self, n):
        return jax.random.permutation(self._next(), n)


kernel_name = 'concat_heads__mha_block_cached__mha_block_cached__near_ridge'

def setup_inputs():
    _rng = _Rng(jax.random.key(int.from_bytes(__import__("os").urandom(4), "little")))
    _w = (lambda a: (lambda t: t.astype(jnp.bfloat16) if jnp.issubdtype(t.dtype, jnp.floating) else t)(jnp.asarray(a)))
    def _A_setup():
        B, Sq, D = 16, 32, 1024
        H, Sk, Dh = 32, 32, 128
        return {
            "x": _w((lambda *s: _rng.normal(s) * 0.8)(B, Sq, D)),
            "k_cache": _w((lambda *s: _rng.normal(s) * 0.8)(B, H, Sk, Dh)),
            "v_cache": _w((lambda *s: _rng.normal(s) * 0.05)(B, H, Sk, Dh)),
            "wq": _w((lambda *s: _rng.normal(s) * 0.8)(D, H * Dh) * (D ** -0.5)),
            "wo": _w((lambda *s: _rng.normal(s) * 0.05)(H * Dh, D) * ((H * Dh) ** -0.5)),
        }
    _A_in = _A_setup()

    def _B_setup():
        B, Sq, D = 16, 32, 1024
        H, Sk, Dh = 32, 32, 128
        return {
            "x": _w((lambda *s: _rng.normal(s) * 0.8)(B, Sq, D)),
            "k_cache": _w((lambda *s: _rng.normal(s) * 0.8)(B, H, Sk, Dh)),
            "v_cache": _w((lambda *s: _rng.normal(s) * 0.05)(B, H, Sk, Dh)),
            "wq": _w((lambda *s: _rng.normal(s) * 0.8)(D, H * Dh) * (D ** -0.5)),
            "wo": _w((lambda *s: _rng.normal(s) * 0.05)(H * Dh, D) * ((H * Dh) ** -0.5)),
        }
    _B_in = _B_setup()

    return {
        "A_x": _A_in["x"],
        "A_k_cache": _A_in["k_cache"],
        "A_v_cache": _A_in["v_cache"],
        "A_wq": _A_in["wq"],
        "A_wo": _A_in["wo"],
        "B_x": _B_in["x"],
        "B_k_cache": _B_in["k_cache"],
        "B_v_cache": _B_in["v_cache"],
        "B_wq": _B_in["wq"],
        "B_wo": _B_in["wo"],
    }

def reference(A_x, A_k_cache, A_v_cache, A_wq, A_wo, B_x, B_k_cache, B_v_cache, B_wq, B_wo):
    def _A_ref(x, k_cache, v_cache, wq, wo):
        B, Sq, D = x.shape
        H, Dh = 32, 128
        q = (lambda x, *d: x.transpose(*d))((x @ wq).reshape(B, Sq, H, Dh), 0, 2, 1, 3)
        scores = jnp.einsum("bhqd,bhkd->bhqk", q, k_cache) * (Dh ** -0.5)
        p = _softmax(scores, axis=-1)
        o = jnp.einsum("bhqk,bhkd->bhqd", p, v_cache)
        return (lambda x, *d: x.transpose(*d))(o, 0, 2, 1, 3).reshape(B, Sq, H * Dh) @ wo

    def _B_ref(x, k_cache, v_cache, wq, wo):
        B, Sq, D = x.shape
        H, Dh = 32, 128
        q = (lambda x, *d: x.transpose(*d))((x @ wq).reshape(B, Sq, H, Dh), 0, 2, 1, 3)
        scores = jnp.einsum("bhqd,bhkd->bhqk", q, k_cache) * (Dh ** -0.5)
        p = _softmax(scores, axis=-1)
        o = jnp.einsum("bhqk,bhkd->bhqd", p, v_cache)
        return (lambda x, *d: x.transpose(*d))(o, 0, 2, 1, 3).reshape(B, Sq, H * Dh) @ wo

    a = _A_ref(A_x, A_k_cache, A_v_cache, A_wq, A_wo)
    b = _B_ref(B_x, B_k_cache, B_v_cache, B_wq, B_wo)
    return jnp.concatenate([a, b], axis=-1)
```

```python
import functools
import jax
import jax.numpy as jnp
from jax import lax
import jax.experimental.pallas as pl
import jax.experimental.pallas.tpu as pltpu

B, SQ, D = 16, 32, 1024
H, SK, DH = 32, 32, 128
M = B * SQ
HH = 16
HW = HH * DH
LOG2E = 1.4426950408889634
SCALE = DH ** -0.5
F32 = jnp.float32
BF16 = jnp.bfloat16


def _scores_softmax(q_ref, k_ref, u, g):
    lane_grp = lax.broadcasted_iota(jnp.int32, (SK, 128), 1) // SQ
    sT = []
    for j in range(4):
        h = 4 * u + j
        kj = k_ref[4 * g:4 * g + 4, h].reshape(128, DH)
        qj = q_ref[128 * g:128 * (g + 1), h * DH:(h + 1) * DH]
        sT.append(lax.dot_general(kj, qj, (((1,), (1,)), ((), ())), preferred_element_type=F32))
    blocks = []
    for c in range(4):
        t = sT[(c - 3) % 4][96:128]
        for b in (2, 1, 0):
            t = jnp.where(lane_grp == b, sT[(c - b) % 4][32 * b:32 * b + 32], t)
        m = jnp.max(t, axis=0, keepdims=True)
        e = jnp.exp2((t - m) * (SCALE * LOG2E))
        l = jnp.sum(e, axis=0, keepdims=True)
        blocks.append(e * (1.0 / l))
    cT = jnp.concatenate(blocks, axis=0)
    return cT.T


def _pv(cm, v_ref, o_ref, u, g):
    row_grp = lax.broadcasted_iota(jnp.int32, (128, 128), 0) // SQ
    col_grp = lax.broadcasted_iota(jnp.int32, (128, 128), 1) // SK
    diff = (col_grp - row_grp) & 3
    for j in range(4):
        h = 4 * u + j
        pj = jnp.where(diff == j, cm, 0.0).astype(BF16)
        vj = jnp.concatenate([v_ref[4 * g + (c - j) % 4, h] for c in range(4)], axis=0)
        o_ref[128 * g:128 * (g + 1), h * DH:(h + 1) * DH] = jnp.dot(pj, vj, preferred_element_type=F32).astype(BF16)


def _build(kchunks=(128, 128, 256, 256, 256), ochunks=(512, 256, 128, 128), lag=1, nosem=True):
    nk = len(kchunks)
    kb = [sum(kchunks[:i]) for i in range(nk + 1)]
    assert kb[-1] == D
    no = len(ochunks)
    ob = [sum(ochunks[:i]) for i in range(no + 1)]
    assert ob[-1] == D

    def kernel(xa, ka, va, wqa, woa, xb, kb_, vb, wqb, wob, out_hbm,
               x_buf, wq_buf, k_buf, v_buf, wo_buf, q_buf, o_buf, qacc, acc, out_buf,
               sem_in, sem_out):
        sem_p = sem_in
        QB = 2 * nk
        AB = QB + 4
        pro = []
        for i in range(nk):
            k0, kn = kb[i], kchunks[i]
            pro.append((
                pltpu.make_async_copy(xa.at[:, pl.ds(k0, kn)], x_buf.at[0, :, pl.ds(k0, kn)], sem_p.at[2 * i]),
                pltpu.make_async_copy(wqa.at[pl.ds(k0, kn), pl.ds(0, HW)], wq_buf.at[0, pl.ds(k0, kn), :], sem_p.at[2 * i + 1])))
        for a, b_ in pro:
            a.start(); b_.start()

        def wq_copy(h):
            src = (wqa, wqb)[h // 2]
            return pltpu.make_async_copy(src.at[:, pl.ds((h % 2) * HW, HW)], wq_buf.at[h], sem_in.at[QB + h])
        cxb = pltpu.make_async_copy(xb, x_buf.at[1], sem_in.at[QB])
        wq_copy(1).start()
        cxb.start()
        wq_copy(2).start()
        wq_copy(3).start()
        for h in range(4):
            k_h, v_h, wo_h = ((ka, va, woa), (kb_, vb, wob))[h // 2]
            o = h % 2
            pltpu.make_async_copy(k_h.at[:, pl.ds(o * HH, HH)], k_buf.at[h], sem_in.at[AB + 3 * h + 0]).start()
            pltpu.make_async_copy(v_h.at[:, pl.ds(o * HH, HH)], v_buf.at[h], sem_in.at[AB + 3 * h + 1]).start()
            pltpu.make_async_copy(wo_h.at[pl.ds(o * HW, HW), :], wo_buf.at[h], sem_in.at[AB + 3 * h + 2]).start()

        for i in range(nk):
            k0, k1 = kb[i], kb[i + 1]
            pro[i][0].wait(); pro[i][1].wait()
            r = jnp.dot(x_buf[0, :, k0:k1], wq_buf[0, k0:k1, :], preferred_element_type=F32)
            if i > 0:
                r = r + qacc[...]
            if i + 1 < nk:
                qacc[...] = r
            else:
                q_buf[0] = r.astype(BF16)

        def qbody(h, carry):
            pltpu.make_async_copy(wqa.at[:, pl.ds(0, HW)], wq_buf.at[h], sem_in.at[QB + h]).wait()

            @pl.when(h == 2)
            def _():
                cxb.wait()
            q_buf[h] = jnp.dot(x_buf[h // 2], wq_buf[h], preferred_element_type=F32).astype(BF16)
            return carry
        lax.fori_loop(1, 4, qbody, 0)

        def out_copy(br, c):
            return pltpu.make_async_copy(out_buf.at[br, :, pl.ds(ob[c], ochunks[c])],
                                         out_hbm.at[:, pl.ds(br * D + ob[c], ochunks[c])], sem_out.at[br, c])

        def abody(h, carry):
            pltpu.make_async_copy(ka.at[:, pl.ds(0, HH)], k_buf.at[h], sem_in.at[AB + 3 * h + 0]).wait()
            pltpu.make_async_copy(va.at[:, pl.ds(0, HH)], v_buf.at[h], sem_in.at[AB + 3 * h + 1]).wait()
            pltpu.make_async_copy(woa.at[pl.ds(0, HW), :], wo_buf.at[h], sem_in.at[AB + 3 * h + 2]).wait()
            br = h // 2
            odd = (h % 2) == 1
            q_ref, k_ref, v_ref = q_buf.at[h], k_buf.at[h], v_buf.at[h]
            cms = {}
            for u in range(4 + lag):
                if u < 4:
                    cms[u] = [_scores_softmax(q_ref, k_ref, u, g) for g in range(4)]
                if u - lag >= 0:
                    for g in range(4):
                        _pv(cms[u - lag][g], v_ref, o_buf, u - lag, g)
            for c in range(no):
                n0, n1 = ob[c], ob[c + 1]
                r = jnp.dot(o_buf[...], wo_buf[h, :, n0:n1], preferred_element_type=F32)
                r = r + jnp.where(odd, acc[:, n0:n1], 0.0)
                acc[:, n0:n1] = r
                out_buf[br, :, n0:n1] = r.astype(BF16)

                @pl.when(odd)
                def _():
                    out_copy(br, c).start()
            return carry
        lax.fori_loop(0, 4, abody, 0)
        for br in range(2):
            for c in range(no):
                out_copy(br, c).wait()

    def fn(A_x, A_k, A_v, A_wq, A_wo, B_x, B_k, B_v, B_wq, B_wo):
        bf = BF16
        out = pl.pallas_call(
            kernel,
            out_shape=jax.ShapeDtypeStruct((M, 2 * D), bf),
            in_specs=[pl.BlockSpec(memory_space=pl.ANY)] * 10,
            out_specs=pl.BlockSpec(memory_space=pl.ANY),
            scratch_shapes=[
                pltpu.VMEM((2, M, D), bf),
                pltpu.VMEM((4, D, HW), bf),
                pltpu.VMEM((4, B, HH, SK, DH), bf),
                pltpu.VMEM((4, B, HH, SK, DH), bf),
                pltpu.VMEM((4, HW, D), bf),
                pltpu.VMEM((4, M, HW), bf),
                pltpu.VMEM((M, HW), bf),
                pltpu.VMEM((M, HW), F32),
                pltpu.VMEM((M, D), F32),
                pltpu.VMEM((2, M, D), bf),
                pltpu.SemaphoreType.DMA((2 * nk + 16,)),
                pltpu.SemaphoreType.DMA((2, no)),
            ],
            compiler_params=pltpu.CompilerParams(vmem_limit_bytes=110 * 1024 * 1024, disable_bounds_checks=True, disable_semaphore_checks=nosem),
        )(A_x.reshape(M, D), A_k, A_v, A_wq, A_wo, B_x.reshape(M, D), B_k, B_v, B_wq, B_wo)
        return out.reshape(B, SQ, 2 * D)
    return fn


_impl = _build()


@jax.jit
def pallas_concat_heads__mha_block_cached__mha_block_cached__near_ridge_kernel(
    A_x: jax.Array,
    A_k_cache: jax.Array,
    A_v_cache: jax.Array,
    A_wq: jax.Array,
    A_wo: jax.Array,
    B_x: jax.Array,
    B_k_cache: jax.Array,
    B_v_cache: jax.Array,
    B_wq: jax.Array,
    B_wo: jax.Array,
):
    return _impl(A_x, A_k_cache, A_v_cache, A_wq, A_wo, B_x, B_k_cache, B_v_cache, B_wq, B_wo)
```

```python
import jax
import jax.numpy as jnp
from jax import lax
import jax.experimental.pallas as pl
import jax.experimental.pallas.tpu as pltpu

B, SQ, D = 16, 32, 1024
H, SK, DH = 32, 32, 128
M = B * SQ
UW = 4 * DH
LOG2E = 1.4426950408889634
SCALE = DH ** -0.5
F32 = jnp.float32
BF16 = jnp.bfloat16
U32 = jnp.uint32

_REGIONS = (
    ((0, 0, 128),),
    ((1, 0, 128), (2, 0, 128), (3, 0, 128)),
    ((0, 128, 256), (1, 128, 256), (2, 128, 256), (3, 128, 256), (4, 0, 128)),
    ((0, 256, 512), (1, 256, 512), (2, 256, 512), (3, 256, 512)),
    ((0, 512, 896), (1, 512, 896), (2, 512, 896), (3, 512, 896)),
    ((0, 896, 1024), (1, 896, 1024), (2, 896, 1024), (3, 896, 1024), (4, 128, 1024), (5, 0, 1024)),
)
_OPIECES = ((0, 512, 0, 512), (512, 768, 0, 512), (768, 1024, 0, 256), (768, 1024, 256, 384),
            (768, 1024, 384, 448), (768, 1024, 448, 512))
_WO_PAD = 128
_O_SLOT, _P_SLOT = 12, 16


def _unit_of(p):
    return 4 * (p // 3) + p % 3


def _plan():
    plan, have = [], 0
    for reg in _REGIONS:
        kmax = max(k1 for _, _, k1 in reg)
        items = []
        if kmax > have:
            items.append((None, have, kmax))
            have = kmax
        plan.append(items + list(reg))
    return plan


_PLAN = _plan()
_S_K0 = sum(len(p) for p in _PLAN)
_S_XB = _S_K0 + 1
_S_Q = _S_XB + 1
_S_A = _S_Q + 6
_NSEM = _S_A + 20


def _u(x):
    return pltpu.bitcast(x, U32)


def _b(x):
    return pltpu.bitcast(x, BF16)


def _dot(a, b):
    return jnp.dot(a, b, preferred_element_type=F32)


def _lane_group(rows):
    return lax.broadcasted_iota(jnp.int32, (rows, 128), 1) // 32


def _sel4(grp, xs):
    t = xs[3]
    for i in (2, 1, 0):
        t = jnp.where(grp == i, xs[i], t)
    return t


def _probs(sts):
    ps = []
    for t in sts:
        m = jnp.max(t, axis=0, keepdims=True)
        e = jnp.exp2((t - m) * (SCALE * LOG2E))
        ps.append(e * (1.0 / jnp.sum(e, axis=0, keepdims=True)))
    return jnp.concatenate(ps, axis=0).T.astype(BF16)


def _mixed(qt, k4, pu, v4):
    g16, g32 = _lane_group(16), _lane_group(32)
    z = jnp.zeros((16, 128), U32)
    qt = [qt[16 * r:16 * r + 16] for r in range(4)]
    k4 = [_u(k) for k in k4]
    v4 = [_u(v) for v in v4]
    outs = []
    for i in range(4):
        w = jnp.concatenate([jnp.where(g16 == i, z, v4[i]) if r == i else jnp.where(g16 != i, z, qt[r])
                             for r in range(4)], axis=0)
        outs.append(_dot(_b(jnp.where(g16 == i, pu, k4[i])), _b(w)))
    ws = jnp.concatenate([jnp.where(g16 != r, z, qt[r]) for r in range(4)], axis=0)
    s_rest = _dot(_b(_sel4(g16, k4)), _b(ws))
    wv = jnp.concatenate([jnp.where(g16 != r, z, v4[r]) for r in range(4)], axis=0)
    o_rest = _dot(_b(pu), _b(wv))
    os_ = [jnp.where(g32 == i, o_rest, outs[i]).astype(BF16) for i in range(4)]
    return _sel4(g32, outs) + s_rest, os_


def _kernel(xa, ka, va, wqa, woa, xb, kb, vb, wqb, wob, out_hbm,
            x_buf, wq_buf, wql_buf, k_buf, v_buf, wo_buf, qop, q_late, qacc, acc, out_buf,
            sem_in, sem_out):
    cp = pltpu.make_async_copy
    wq_h, k_h, v_h, wo_h = (wqa, wqb), (ka, kb), (va, vb), (woa, wob)

    pro, s = [], 0
    for items in _PLAN:
        cur = []
        for p, k0, k1 in items:
            ks = pl.ds(k0, k1 - k0)
            if p is None:
                cur.append(cp(xa.at[:, ks], x_buf.at[0, :, ks], sem_in.at[s]))
            else:
                cur.append(cp(wqa.at[ks, pl.ds(_unit_of(p) * UW, UW)], wq_buf.at[p, ks, :], sem_in.at[s]))
            s += 1
        pro.append(cur)
    pro[-1].append(cp(ka.at[:, pl.ds(0, 4)], k_buf.at[0, :, pl.ds(0, 4)], sem_in.at[_S_K0]))
    cxb = cp(xb, x_buf.at[1], sem_in.at[_S_XB])

    def q_copy(src_unit, p):
        return cp(wqb.at[:, pl.ds(src_unit * UW, UW)], wq_buf.at[p], sem_in.at[_S_Q + p - 6])

    def main_copies(src, par, h, br):
        sb, h0 = _S_A + 5 * h, 16 * par
        return [
            cp(wq_h[src].at[:, pl.ds((4 * par + 3) * UW, UW)], wql_buf.at[h], sem_in.at[sb]),
            cp(k_h[src].at[:, pl.ds(h0 + 4, 12)], k_buf.at[br, :, pl.ds(h0 + 4, 12)], sem_in.at[sb + 1]),
            cp(v_h[src].at[:, pl.ds(h0, 16)], v_buf.at[br, :, pl.ds(h0, 16)], sem_in.at[sb + 2]),
            cp(wo_h[src].at[pl.ds(4 * par, 4)], wo_buf.at[pl.ds(4 * h, 4), :, pl.ds(0, D)], sem_in.at[sb + 3]),
        ]

    def next_k_copy(src, npar, h, nbr):
        hs = pl.ds(16 * npar, 4)
        return cp(k_h[src].at[:, hs], k_buf.at[nbr, :, hs], sem_in.at[_S_A + 5 * h + 4])

    for cur in pro:
        for c in cur:
            c.start()
    cxb.start()
    for p in range(6, 12):
        q_copy(_unit_of(p) - 8, p).start()
    for h in range(4):
        for c in main_copies(h // 2, h % 2, h, h // 2):
            c.start()
        if h < 3:
            next_k_copy((h + 1) // 2, (h + 1) % 2, h, (h + 1) // 2).start()

    def p_block(step, g):
        return qop.at[_P_SLOT, pl.ds(128 * step, 128), pl.ds(128 * g, 128)]

    for ri, reg in enumerate(_REGIONS):
        for c in pro[ri]:
            c.wait()
        for ji, (p, k0, k1) in enumerate(reg):
            r = _dot(x_buf[0, :, k0:k1], wq_buf[p, k0:k1, :])
            if k0 > 0:
                r = r + qacc[p]
            if k1 < D:
                qacc[p] = r
            else:
                qop[p] = r.astype(BF16)
            if ri == len(_REGIONS) - 1 and ji == len(reg) - 2:
                g32 = _lane_group(32)
                for g in range(4):
                    sts = []
                    for j in range(4):
                        kk = k_buf[0, 4 * g:4 * g + 4, j].reshape(128, DH)
                        qq = qop[0, 128 * g:128 * g + 128, j * DH:(j + 1) * DH]
                        full = lax.dot_general(kk, qq, (((1,), (1,)), ((), ())), preferred_element_type=F32)
                        sts.append(_sel4(g32, [full[32 * i:32 * i + 32] for i in range(4)]))
                    p_block(0, g)[...] = _probs(sts)

    cxb.wait()

    def q_body(it, carry):
        for c in range(3):
            q_copy(4 * it + c, 6 + 3 * it + c).wait()
        for c in range(3):
            p = 6 + 3 * it + c
            qop[p] = _dot(x_buf[1], wq_buf[p]).astype(BF16)
        return carry
    lax.fori_loop(0, 2, q_body, 0)

    def out_copy(br, c):
        n0, n1, m0, m1 = _OPIECES[c]
        rows = pl.ds(m0, m1 - m0)
        return cp(out_buf.at[br, rows, pl.ds(n0, n1 - n0)],
                  out_hbm.at[rows, pl.ds(br * D + n0, n1 - n0)], sem_out.at[br, c])

    def main_body(h, carry):
        br, par = lax.shift_right_logical(h, 1), h & 1
        hn = jnp.minimum(h + 1, 3)
        nbr, npar = lax.shift_right_logical(hn, 1), hn & 1
        for c in main_copies(0, par, h, br):
            c.wait()

        @pl.when(h < 3)
        def _():
            next_k_copy(0, npar, h, nbr).wait()
        h0 = 16 * par
        second_half = par == 1

        def oproj(s, n0, n1, m0=0, m1=M):
            r = _dot(qop[_O_SLOT + s, m0:m1, :], wo_buf[4 * h + s, :, n0:n1])
            if s == 0:
                r = r + jnp.where(second_half, acc[m0:m1, n0:n1], 0.0)
            else:
                r = r + acc[m0:m1, n0:n1]
            acc[m0:m1, n0:n1] = r
            if s == 3:
                out_buf[br, m0:m1, n0:n1] = r.astype(BF16)

        for s in range(4):
            if s < 2:
                q_ref, sbr, sh = qop.at[3 * h + s + 1], br, h0 + 4 * (s + 1)
            elif s == 2:
                q_ref, sbr, sh = q_late, br, h0 + 12
            else:
                q_ref, sbr, sh = qop.at[3 * hn], nbr, 16 * npar
            for g in range(4):
                if s == 0:
                    cols = slice(128 * g, 128 * g + 128)
                    q_late[:, cols] = _dot(x_buf[br], wql_buf[h, :, cols]).astype(BF16)
                else:
                    oproj(s - 1, 256 * g, 256 * g + 256)
                pu = _u(p_block(s, g)[...])
                qts = [_u(q_ref[128 * g:128 * g + 128, j * DH:(j + 1) * DH].T) for j in range(4)]
                sts = []
                for j in range(4):
                    bo = 4 * g + j
                    st, os_ = _mixed(qts[j],
                                     [k_buf[sbr, 4 * g + i, sh + j] for i in range(4)],
                                     pu[16 * j:16 * j + 16],
                                     [v_buf[br, bo, h0 + 4 * s + i] for i in range(4)])
                    for i in range(4):
                        qop[_O_SLOT + s, 32 * bo:32 * bo + 32, i * DH:(i + 1) * DH] = os_[i]
                    sts.append(st)
                p_block((s + 1) % 4, g)[...] = _probs(sts)
        for c in range(len(_OPIECES)):
            oproj(3, *_OPIECES[c])

            @pl.when(second_half)
            def _():
                out_copy(br, c).start()
        return carry
    lax.fori_loop(0, 4, main_body, 0)
    for br in range(2):
        for c in range(len(_OPIECES)):
            out_copy(br, c).wait()


@jax.jit
def pallas_concat_heads__mha_block_cached__mha_block_cached__near_ridge_kernel(
    A_x: jax.Array,
    A_k_cache: jax.Array,
    A_v_cache: jax.Array,
    A_wq: jax.Array,
    A_wo: jax.Array,
    B_x: jax.Array,
    B_k_cache: jax.Array,
    B_v_cache: jax.Array,
    B_wq: jax.Array,
    B_wo: jax.Array,
):
    out = pl.pallas_call(
        _kernel,
        out_shape=jax.ShapeDtypeStruct((M, 2 * D), BF16),
        in_specs=[pl.BlockSpec(memory_space=pl.ANY)] * 10,
        out_specs=pl.BlockSpec(memory_space=pl.ANY),
        scratch_shapes=[
            pltpu.VMEM((2, M, D), BF16),
            pltpu.VMEM((12, D, UW), BF16),
            pltpu.VMEM((4, D, UW), BF16),
            pltpu.VMEM((2, B, H, SK, DH), BF16),
            pltpu.VMEM((2, B, H, SK, DH), BF16),
            pltpu.VMEM((16, UW, D + _WO_PAD), BF16),
            pltpu.VMEM((17, M, UW), BF16),
            pltpu.VMEM((M, UW), BF16),
            pltpu.VMEM((5, M, UW), F32),
            pltpu.VMEM((M, D), F32),
            pltpu.VMEM((2, M, D), BF16),
            pltpu.SemaphoreType.DMA((_NSEM,)),
            pltpu.SemaphoreType.DMA((2, len(_OPIECES))),
        ],
        compiler_params=pltpu.CompilerParams(
            vmem_limit_bytes=110 * 1024 * 1024,
            disable_bounds_checks=True,
            disable_semaphore_checks=True,
        ),
    )(A_x.reshape(M, D), A_k_cache, A_v_cache, A_wq, A_wo.reshape(8, UW, D),
      B_x.reshape(M, D), B_k_cache, B_v_cache, B_wq, B_wo.reshape(8, UW, D))
    return out.reshape(B, SQ, 2 * D)
```

```python
import jax
import jax.numpy as jnp
from jax import lax
import jax.experimental.pallas as pl
import jax.experimental.pallas.tpu as pltpu

B, SQ, D = 16, 32, 1024
H, SK, DH = 32, 32, 128
M = B * SQ
UW = 4 * DH
LOG2E = 1.4426950408889634
SCALE = DH ** -0.5
F32 = jnp.float32
BF16 = jnp.bfloat16
U32 = jnp.uint32

_REGIONS = (
    ((0, 0, 128),),
    ((1, 0, 128), (2, 0, 128), (3, 0, 128)),
    ((4, 0, 128), (5, 0, 128), (0, 128, 256), (1, 128, 256)),
    ((2, 128, 384), (3, 128, 384), (4, 128, 256), (5, 128, 256), (0, 256, 384), (1, 256, 384)),
    ((4, 256, 640), (5, 256, 512), (0, 384, 640), (1, 384, 640), (2, 384, 640), (3, 384, 640)),
    ((0, 640, 1024), (1, 640, 1024), (2, 640, 1024), (3, 640, 1024), (4, 640, 1024), (5, 512, 1024)),
)
_OPIECES = ((0, 512, 0, 512), (512, 768, 0, 512), (768, 1024, 0, 256), (768, 1024, 256, 384),
            (768, 1024, 384, 448), (768, 1024, 448, 512))
_WO_PAD = 128
_O_SLOT = 12
_QO_SLOTS = 18


def _unit_of(p):
    return 4 * (p // 3) + p % 3


def _plan():
    plan, have = [], 0
    for reg in _REGIONS:
        kmax = max(k1 for _, _, k1 in reg)
        items = []
        if kmax > have:
            items.append((None, have, kmax))
            have = kmax
        plan.append(items + list(reg))
    return plan


_PLAN = _plan()
_S_Q = len(_PLAN)
_S_A = _S_Q + 2
_S_X = _S_A + 4
_NSEM = _S_X + 1


def _u(x):
    return pltpu.bitcast(x, U32)


def _b(x):
    return pltpu.bitcast(x, BF16)


def _dot(a, b):
    return jnp.dot(a, b, preferred_element_type=F32)


def _lane_group(rows):
    return lax.broadcasted_iota(jnp.int32, (rows, 128), 1) // 32


def _sel4(grp, xs):
    t = xs[3]
    for i in (2, 1, 0):
        t = jnp.where(grp == i, xs[i], t)
    return t


def _probs(sts):
    ps = []
    for t in sts:
        m = jnp.max(t, axis=0, keepdims=True)
        e = jnp.exp2((t - m) * (SCALE * LOG2E))
        ps.append(e * (1.0 / jnp.sum(e, axis=0, keepdims=True)))
    return jnp.concatenate(ps, axis=0).T.astype(BF16)


def _mixed(qt, k4, pu, v4):
    g16, g32 = _lane_group(16), _lane_group(32)
    z = jnp.zeros((16, 128), U32)
    qt = [qt[16 * r:16 * r + 16] for r in range(4)]
    k4 = [_u(k) for k in k4]
    v4 = [_u(v) for v in v4]
    outs = []
    for i in range(4):
        w = jnp.concatenate([jnp.where(g16 == i, z, v4[i]) if r == i else jnp.where(g16 != i, z, qt[r])
                             for r in range(4)], axis=0)
        outs.append(_dot(_b(jnp.where(g16 == i, pu, k4[i])), _b(w)))
    ws = jnp.concatenate([jnp.where(g16 != r, z, qt[r]) for r in range(4)], axis=0)
    s_rest = _dot(_b(_sel4(g16, k4)), _b(ws))
    wv = jnp.concatenate([jnp.where(g16 != r, z, v4[r]) for r in range(4)], axis=0)
    o_rest = _dot(_b(pu), _b(wv))
    os_ = [jnp.where(g32 == i, o_rest, outs[i]).astype(BF16) for i in range(4)]
    return _sel4(g32, outs) + s_rest, os_


def _kernel(xa, ka, va, wqa, woa, xb, kb, vb, wqb, wob, out_hbm,
            x_buf, wq_buf, wql_buf, k_buf, k_spare, v_buf, wo_buf, qo, p_buf, q_late, qacc, acc, out_buf,
            sem_in, sem_out):
    cp = pltpu.make_async_copy
    wq_h, k_h, v_h, wo_h = (wqa, wqb), (ka, kb), (va, vb), (woa, wob)

    def wait_kib(kib, sem):
        a = next(a for a in range(1, _QO_SLOTS + 1) if kib % a == 0 and kib // a <= M and (kib // a) % 16 == 0)
        view = qo.at[pl.ds(0, a), pl.ds(0, kib // a)]
        cp(view, view, sem).wait()

    def k_first(h, sem):
        b4, hs = pl.ds(0, 4), pl.ds(16 * (h % 2), 4)
        return cp(k_h[h // 2].at[b4, hs], k_buf.at[h // 2, b4, hs], sem)

    pro_kib = []
    for s, items in enumerate(_PLAN):
        for p, k0, k1 in items:
            ks = pl.ds(k0, k1 - k0)
            if p is None:
                cp(xa.at[:, ks], x_buf.at[0, :, ks], sem_in.at[s]).start()
            else:
                cp(wqa.at[ks, pl.ds(_unit_of(p) * UW, UW)], wq_buf.at[p, ks, :], sem_in.at[s]).start()
        pro_kib.append(sum(k1 - k0 for _, k0, k1 in items))
    k_first(0, sem_in.at[len(_PLAN) - 1]).start()
    pro_kib[-1] += 128

    xb_copy = cp(xb, x_buf.at[1], sem_in.at[_S_X])
    xb_copy.start()
    for p in range(6, 12):
        cp(wqb.at[:, pl.ds((_unit_of(p) - 8) * UW, UW)], wq_buf.at[p], sem_in.at[_S_Q + (p - 6) // 3]).start()

    for h in range(4):
        br, par = h // 2, h % 2
        sem, h0 = sem_in.at[_S_A + h], 16 * par
        b12, hs = pl.ds(4, 12), pl.ds(h0, 4)
        cp(wq_h[br].at[:, pl.ds((4 * par + 3) * UW, UW)], wql_buf.at[h], sem).start()
        cp(k_h[br].at[b12, hs], k_buf.at[br, b12, hs], sem).start()
        cp(k_h[br].at[:, pl.ds(h0 + 4, 12)], k_buf.at[br, :, pl.ds(h0 + 4, 12)], sem).start()
        cp(v_h[br].at[:, pl.ds(h0, 16)], v_buf.at[br, :, pl.ds(h0, 16)], sem).start()
        cp(wo_h[br].at[pl.ds(4 * par, 4)], wo_buf.at[pl.ds(4 * h, 4), :, pl.ds(0, D)], sem).start()
        if h < 3:
            k_first(h + 1, sem).start()
        else:
            cp(ka.at[pl.ds(0, 4), pl.ds(0, 4)], k_spare, sem).start()

    for ri, reg in enumerate(_REGIONS):
        wait_kib(pro_kib[ri], sem_in.at[ri])
        for ji, (p, k0, k1) in enumerate(reg):
            r = _dot(x_buf[0, :, k0:k1], wq_buf[p, k0:k1, :])
            if k0 > 0:
                r = r + qacc[p]
            if k1 < D:
                qacc[p] = r
            else:
                qo[p] = r.astype(BF16)
            if ri == len(_REGIONS) - 1 and ji == len(reg) - 2:
                g32 = _lane_group(32)
                sts = []
                for j in range(4):
                    kk = k_buf[0, 0:4, j].reshape(128, DH)
                    qq = qo[0, 0:128, j * DH:(j + 1) * DH]
                    full = lax.dot_general(kk, qq, (((1,), (1,)), ((), ())), preferred_element_type=F32)
                    sts.append(_sel4(g32, [full[32 * i:32 * i + 32] for i in range(4)]))
                p_buf[0, 0] = _probs(sts)

    xb_copy.wait()

    def q_body(it, carry):
        wait_kib(3072, sem_in.at[_S_Q + it])
        for c in range(3):
            p = 6 + 3 * it + c
            qo[p] = _dot(x_buf[1], wq_buf[p]).astype(BF16)
        return carry
    lax.fori_loop(0, 2, q_body, 0)

    def out_copy(br, c):
        n0, n1, m0, m1 = _OPIECES[c]
        rows = pl.ds(m0, m1 - m0)
        return cp(out_buf.at[br, rows, pl.ds(n0, n1 - n0)],
                  out_hbm.at[rows, pl.ds(br * D + n0, n1 - n0)], sem_out.at[br, c])

    def main_body(h, carry):
        wait_kib(9216, sem_in.at[_S_A + h])
        br, par = lax.shift_right_logical(h, 1), h & 1
        hn = jnp.minimum(h + 1, 3)
        nbr, npar = lax.shift_right_logical(hn, 1), hn & 1
        h0 = 16 * par
        second_half = par == 1

        def oproj(s, n0, n1, m0=0, m1=M):
            r = _dot(qo[_O_SLOT + s, m0:m1, :], wo_buf[4 * h + s, :, n0:n1])
            if s == 0:
                r = r + jnp.where(second_half, acc[m0:m1, n0:n1], 0.0)
            else:
                r = r + acc[m0:m1, n0:n1]
            acc[m0:m1, n0:n1] = r
            if s == 3:
                out_buf[br, m0:m1, n0:n1] = r.astype(BF16)

        def score_side(s):
            if s < 3:
                return qo.at[3 * h + s], br, h0 + 4 * s
            if s == 3:
                return q_late, br, h0 + 12
            return qo.at[3 * hn], nbr, 16 * npar

        for s in range(4):
            for g in range(4):
                if s == 0:
                    cols = slice(128 * g, 128 * g + 128)
                    q_late[:, cols] = _dot(x_buf[br], wql_buf[h, :, cols]).astype(BF16)
                else:
                    oproj(s - 1, 256 * g, 256 * g + 256)
                ns, ng = (s, g + 1) if g < 3 else (s + 1, 0)
                q_ref, sbr, sh = score_side(ns)
                pu = _u(p_buf[s, g])
                qts = [_u(q_ref[128 * ng:128 * ng + 128, j * DH:(j + 1) * DH].T) for j in range(4)]
                sts = []
                for j in range(4):
                    bo = 4 * g + j
                    st, os_ = _mixed(qts[j],
                                     [k_buf[sbr, 4 * ng + i, sh + j] for i in range(4)],
                                     pu[16 * j:16 * j + 16],
                                     [v_buf[br, bo, h0 + 4 * s + i] for i in range(4)])
                    for i in range(4):
                        qo[_O_SLOT + s, 32 * bo:32 * bo + 32, i * DH:(i + 1) * DH] = os_[i]
                    sts.append(st)
                p_buf[ns % 4, ng] = _probs(sts)
        for c in range(len(_OPIECES)):
            oproj(3, *_OPIECES[c])

            @pl.when(second_half)
            def _():
                out_copy(br, c).start()
        return carry
    lax.fori_loop(0, 4, main_body, 0)
    for br in range(2):
        for c in range(len(_OPIECES)):
            out_copy(br, c).wait()


@jax.jit
def pallas_concat_heads__mha_block_cached__mha_block_cached__near_ridge_kernel(
    A_x: jax.Array,
    A_k_cache: jax.Array,
    A_v_cache: jax.Array,
    A_wq: jax.Array,
    A_wo: jax.Array,
    B_x: jax.Array,
    B_k_cache: jax.Array,
    B_v_cache: jax.Array,
    B_wq: jax.Array,
    B_wo: jax.Array,
):
    out = pl.pallas_call(
        _kernel,
        out_shape=jax.ShapeDtypeStruct((M, 2 * D), BF16),
        in_specs=[pl.BlockSpec(memory_space=pl.ANY)] * 10,
        out_specs=pl.BlockSpec(memory_space=pl.ANY),
        scratch_shapes=[
            pltpu.VMEM((2, M, D), BF16),
            pltpu.VMEM((12, D, UW), BF16),
            pltpu.VMEM((4, D, UW), BF16),
            pltpu.VMEM((2, B, H, SK, DH), BF16),
            pltpu.VMEM((4, 4, SK, DH), BF16),
            pltpu.VMEM((2, B, H, SK, DH), BF16),
            pltpu.VMEM((16, UW, D + _WO_PAD), BF16),
            pltpu.VMEM((_QO_SLOTS, M, UW), BF16),
            pltpu.VMEM((4, 4, 128, 128), BF16),
            pltpu.VMEM((M, UW), BF16),
            pltpu.VMEM((6, M, UW), F32),
            pltpu.VMEM((M, D), F32),
            pltpu.VMEM((2, M, D), BF16),
            pltpu.SemaphoreType.DMA((_NSEM,)),
            pltpu.SemaphoreType.DMA((2, len(_OPIECES))),
        ],
        compiler_params=pltpu.CompilerParams(
            vmem_limit_bytes=110 * 1024 * 1024,
            disable_bounds_checks=True,
            disable_semaphore_checks=True,
        ),
    )(A_x.reshape(M, D), A_k_cache, A_v_cache, A_wq, A_wo.reshape(8, UW, D),
      B_x.reshape(M, D), B_k_cache, B_v_cache, B_wq, B_wo.reshape(8, UW, D))
    return out.reshape(B, SQ, 2 * D)
```
